```python
import jax
import jax.numpy as jnp

def _softmax(x, axis=-1):
    return jax.nn.softmax(x, axis=axis)

def _gelu(x):
    return jax.nn.gelu(x, approximate=True)

def _silu(x):
    return jax.nn.silu(x)

def _sigmoid(x):
    return jax.nn.sigmoid(x)

def _layernorm(x, axis=-1, eps=1e-05):
    m = jnp.mean(x, axis=axis, keepdims=True)
    v = jnp.var(x, axis=axis, keepdims=True)
    return (x - m) / jnp.sqrt(v + eps)

def _scatter_add(tgt, idx, src, axis=0):
    return tgt.at[idx].add(src)

def _segment_sum(src, seg, n):
    return jax.ops.segment_sum(src, seg, n)

class _Rng:

    def __init__(self, key):
        self._k = key

    def _next(self):
        self._k, sub = jax.random.split(self._k)
        return sub

    def normal(self, shape):
        return jax.random.normal(self._next(), shape, dtype=jnp.bfloat16)

    def randint(self, lo, hi, shape):
        return jax.random.randint(self._next(), shape, lo, hi, dtype=jnp.int32)

    def uniform(self, shape, lo=0.0, hi=1.0):
        return jax.random.uniform(self._next(), shape, jnp.bfloat16, lo, hi)

    def permutation(self, n):
        return jax.random.permutation(self._next(), n)
kernel_name = 'adaLN_cond__sliding_block_cached__glu_gated_swiglu__decode'

def setup_inputs():
    _rng = _Rng(jax.random.key(int.from_bytes(__import__("os").urandom(4), "little")))
    _w = lambda a: (lambda t: t.astype(jnp.bfloat16) if jnp.issubdtype(t.dtype, jnp.floating) else t)(jnp.asarray(a))

    def _A_setup():
        B, Sq, D = (2, 1, 512)
        Hq, Hkv, Sk, Dh = (32, 32, 16384, 128)
        assert Hq % Hkv == 0, (Hq, Hkv)
        return {'x': _w((lambda *s: _rng.normal(s) * 0.05)(B, Sq, D)), 'k_cache': _w((lambda *s: _rng.normal(s) * 0.05)(B, Hkv, Sk, Dh)), 'v_cache': _w((lambda *s: _rng.normal(s) * 0.05)(B, Hkv, Sk, Dh)), 'wq': _w((lambda *s: _rng.normal(s) * 0.05)(D, Hq * Dh) * D ** (-0.5)), 'wo': _w((lambda *s: _rng.normal(s) * 0.05)(Hq * Dh, D) * (Hq * Dh) ** (-0.5))}
    _A_in = _A_setup()

    def _B_setup():
        B, S, D, F = (2, 1, 512, 1376)
        return {'x': _w((lambda *s: _rng.normal(s) * 0.05)(B, S, D)), 'w1': _w((lambda *s: _rng.normal(s) * 0.05)(D, F) * (2.0 / D) ** 0.5), 'w3': _w((lambda *s: _rng.normal(s) * 0.05)(D, F) * (2.0 / D) ** 0.5), 'w2': _w((lambda *s: _rng.normal(s) * 0.05)(F, D) * (2.0 / F) ** 0.5)}
    _B_in = _B_setup()
    return {'A_x': _A_in['x'], 'A_k_cache': _A_in['k_cache'], 'A_v_cache': _A_in['v_cache'], 'A_wq': _A_in['wq'], 'A_wo': _A_in['wo'], 'B_x': _B_in['x'], 'B_w1': _B_in['w1'], 'B_w3': _B_in['w3'], 'B_w2': _B_in['w2'], 'c': _w((lambda *s: _rng.normal(s) * 0.05)(2, 512)), 'w_mod': _w((lambda *s: _rng.normal(s) * 0.05)(512, 6 * 512) * 512 ** (-0.5))}

def reference(A_x, A_k_cache, A_v_cache, A_wq, A_wo, B_x, B_w1, B_w3, B_w2, c, w_mod):

    def _A_ref(x, k_cache, v_cache, wq, wo):
        B, Sq, D = x.shape
        Hq, Dh = (32, 128)
        Hkv, Sk = (k_cache.shape[1], k_cache.shape[2])
        W = min(4096, max(256, Sk // 4))
        rep = Hq // Hkv
        q = (lambda x, *d: x.transpose(*d))((x @ wq).reshape(B, Sq, Hq, Dh), 0, 2, 1, 3)
        k = jnp.repeat(k_cache[:, :, Sk - W:, :], rep, axis=1)
        v = jnp.repeat(v_cache[:, :, Sk - W:, :], rep, axis=1)
        scores = jnp.einsum('bhqd,bhkd->bhqk', q, k) * Dh ** (-0.5)
        p = _softmax(scores, axis=-1)
        o = jnp.einsum('bhqk,bhkd->bhqd', p, v)
        return (lambda x, *d: x.transpose(*d))(o, 0, 2, 1, 3).reshape(B, Sq, Hq * Dh) @ wo

    def _B_ref(x, w1, w3, w2):
        gate = jnp.einsum('bsd,df->bsf', x, w1)
        up = jnp.einsum('bsd,df->bsf', x, w3)
        h = _silu(gate) * up
        out = jnp.einsum('bsf,fd->bsd', h, w2)
        return out
    x = A_x
    mod = (_silu(c) @ w_mod).reshape(c.shape[0], 6, 1, -1)
    sa, ca, ga, sb, cb, gb = (mod[:, 0].copy(), mod[:, 1].copy(), mod[:, 2].copy(), mod[:, 3].copy(), mod[:, 4].copy(), mod[:, 5].copy())
    h = _layernorm(x, axis=-1) * (1 + ca) + sa
    x = x + ga * _A_ref(h, A_k_cache, A_v_cache, A_wq, A_wo)
    h = _layernorm(x, axis=-1) * (1 + cb) + sb
    x = x + gb * _B_ref(h, B_w1, B_w3, B_w2)
    return x
```

```python
import jax
import jax.numpy as jnp
import jax.experimental.pallas as pl
import jax.experimental.pallas.tpu as pltpu

NT = (((1,), (1,)), ((), ()))
f32 = jnp.float32
bf16 = jnp.bfloat16


def _ln(x, eps=1e-5):
    m = jnp.mean(x, axis=-1, keepdims=True)
    d = x - m
    v = jnp.mean(d * d, axis=-1, keepdims=True)
    return d / jnp.sqrt(v + eps)


def _spread(n, ways):
    per = -(-n // ways)
    return [w * per + j for j in range(per) for w in range(ways) if w * per + j < n]


def make(G=8, R=512, piece=128, rot=0, wways=8, wbytes=32768, checks=False, w2split=1280):
    def kernel(x_hbm, k_hbm, v_hbm, wq_hbm, wo_hbm, w1_hbm, w3_hbm, w2_hbm, c_hbm, wm_hbm,
               o_ref,
               xv, cv, wmv, wqv, wov, w1v, w3v, w2v, kbuf, vbuf, qs, ss, ps, acc, os_,
               wsem, ksem, vsem):
        BH, SK, DH = k_hbm.shape
        B, D = xv.shape
        H = BH // B
        NC = kbuf.shape[0]
        W = NC * R
        NG = BH // G
        F = w2v.shape[0]
        cnt = [0]

        def start_w(src, dst, sem, r0=0, r1=None, c0=0, c1=None):
            r1 = src.shape[0] if r1 is None else r1
            c1 = src.shape[1] if c1 is None else c1
            cols = c1 - c0
            rows = 16
            while rows * cols * 2 < wbytes:
                rows *= 2
            csz = min(cols, wbytes // (rows * 2))
            pieces = [(r, min(rows, r1 - r), c) for r in range(r0, r1, rows) for c in range(c0, c1, csz)]
            for i in _spread(len(pieces), wways):
                r, nr, c = pieces[i]
                pltpu.make_async_copy(src.at[pl.ds(r, nr), pl.ds(c, csz)],
                                      dst.at[pl.ds(r, nr), pl.ds(c, csz)], sem).start(priority=cnt[0] % 2)
                cnt[0] += 1

        def wait(dst, sem):
            pltpu.make_async_copy(dst, dst, sem).wait()

        def start_chunk(hbm, buf, sem, g, c):
            npc = R // piece
            for j in range(npc):
                for w in range(G):
                    r = ((j + w * rot) % npc) * piece
                    pltpu.make_async_copy(
                        hbm.at[g * G + w, pl.ds(pl.multiple_of(SK - W + c * R + r, piece), piece)],
                        buf.at[c, w, pl.ds(r, piece)], sem.at[c]).start(priority=w % 2)

        cc = pltpu.make_async_copy(c_hbm, cv, wsem.at[0])
        cx = pltpu.make_async_copy(x_hbm, xv, wsem.at[1])
        cc.start()
        cx.start(priority=1)
        start_w(wm_hbm, wmv, wsem.at[2])
        start_w(wq_hbm, wqv, wsem.at[3], 0, D // 2)
        cc.wait()
        cx.wait()
        wait(wmv, wsem.at[2])
        cf = cv[...].astype(f32)
        sc = (cf * jax.nn.sigmoid(cf)).astype(bf16)
        mod = jnp.dot(sc, wmv[...], preferred_element_type=f32)
        sa, ca, ga, sb, cb, gb = [mod[:, j * D:(j + 1) * D] for j in range(6)]
        x = xv[...].astype(f32)
        hh = (_ln(x) * (1.0 + ca) + sa).astype(bf16)
        start_w(wq_hbm, wqv, wsem.at[3], D // 2, D)
        for c in range(3):
            start_chunk(k_hbm, kbuf, ksem, 0, c)
        wait(wqv, wsem.at[3])
        q = jnp.dot(hh, wqv[...], preferred_element_type=f32)
        for b in range(B):
            for h in range(H):
                i = b * H + h
                qs[i // G, pl.ds(i % G, 1), :] = q[b:b + 1, h * DH:(h + 1) * DH]
        for c in range(3, NC):
            start_chunk(k_hbm, kbuf, ksem, 0, c)

        scale = DH ** -0.5
        row = jax.lax.broadcasted_iota(jnp.int32, (G, DH), 0)

        def k_phase(g):
            qg = qs[g]
            qw = [jnp.where(row == w, qg, 0.0).astype(bf16) for w in range(G)]

            def body(c, carry):
                start_chunk(v_hbm, vbuf, vsem, g, c)
                wait(kbuf.at[c], ksem.at[c])
                s = None
                for w in range(G):
                    t = jax.lax.dot_general(qw[w], kbuf[c, w], NT, preferred_element_type=f32)
                    s = t if s is None else s + t
                ss[c] = s * scale
                return carry

            jax.lax.fori_loop(0, NC, body, 0)
            s = ss[...]
            m = jnp.max(jnp.max(s, axis=0), axis=-1, keepdims=True)
            p = jnp.exp(s - m)
            l = jnp.sum(jnp.sum(p, axis=0), axis=-1, keepdims=True)
            ps[...] = p.astype(bf16)
            acc[...] = jnp.zeros(acc.shape, f32)
            return l

        def pv(c):
            wait(vbuf.at[c], vsem.at[c])
            p = ps[c]
            t = acc[...]
            for w in range(G):
                o = jnp.dot(p, vbuf[c, w], preferred_element_type=f32)
                t = t + jnp.where(row == w, o, 0.0)
            acc[...] = t

        def group(g, carry):
            l = k_phase(g)

            def body(c, carry):
                start_chunk(k_hbm, kbuf, ksem, g + 1, c)
                pv(c)
                return carry

            jax.lax.fori_loop(0, NC, body, 0)
            os_[g] = acc[...] / l
            return carry

        jax.lax.fori_loop(0, NG - 1, group, 0)

        l = k_phase(NG - 1)
        HD = H * DH
        nq = 4
        for j in range(nq):
            start_w(wo_hbm, wov, wsem.at[4 + (j == nq - 1)], j * HD // nq, (j + 1) * HD // nq)
            for c in range(j * NC // nq, (j + 1) * NC // nq):
                pv(c)
        os_[NG - 1] = acc[...] / l
        start_w(w1_hbm, w1v, wsem.at[6])
        brow = jax.lax.broadcasted_iota(jnp.int32, (8, DH), 0)
        cols = []
        for h in range(H):
            t = jnp.zeros((8, DH), f32)
            for b in range(B):
                i = b * H + h
                t = jnp.where(brow == b, os_[i // G, pl.ds(i % G, 1), :], t)
            cols.append(t.astype(bf16))
        k0 = (nq - 1) * HD // nq
        wait(wov.at[pl.ds(0, k0)], wsem.at[4])
        a = jnp.dot(jnp.concatenate(cols[:k0 // DH], axis=-1), wov[0:k0, :], preferred_element_type=f32)
        start_w(w3_hbm, w3v, wsem.at[7])
        wait(wov.at[pl.ds(k0, HD - k0)], wsem.at[5])
        a = a + jnp.dot(jnp.concatenate(cols[k0 // DH:], axis=-1), wov[k0:HD, :], preferred_element_type=f32)
        x1 = x + ga * a[0:B]
        h2 = (_ln(x1) * (1.0 + cb) + sb).astype(bf16)
        start_w(w2_hbm, w2v, wsem.at[8], 0, w2split)
        start_w(w2_hbm, w2v, wsem.at[9], w2split, F)
        wait(w1v, wsem.at[6])
        gt = jax.lax.dot_general(h2, w1v[...], NT, preferred_element_type=f32)
        gt = gt * jax.nn.sigmoid(gt)
        wait(w3v, wsem.at[7])
        u = jax.lax.dot_general(h2, w3v[...], NT, preferred_element_type=f32)
        hf = (gt * u).astype(bf16)
        wait(w2v.at[pl.ds(0, w2split)], wsem.at[8])
        y = jnp.dot(hf[:, :w2split], w2v[0:w2split, :], preferred_element_type=f32)
        wait(w2v.at[pl.ds(w2split, F - w2split)], wsem.at[9])
        y = y + jnp.dot(hf[:, w2split:], w2v[w2split:F, :], preferred_element_type=f32)
        o_ref[...] = (x1 + gb * y).astype(o_ref.dtype)

    def f(A_x, A_k_cache, A_v_cache, A_wq, A_wo, B_x, B_w1, B_w3, B_w2, c, w_mod):
        B, Sq, D = A_x.shape
        _, H, SK, DH = A_k_cache.shape
        W = min(4096, max(256, SK // 4))
        F = B_w1.shape[1]
        NC = W // R
        NG = B * H // G
        args = [A_x.reshape(B, D), A_k_cache.reshape(B * H, SK, DH), A_v_cache.reshape(B * H, SK, DH),
                A_wq, A_wo, B_w1.T, B_w3.T, B_w2, c, w_mod]
        args = [pltpu.with_memory_space_constraint(a, pltpu.HBM) for a in args]
        out = pl.pallas_call(
            kernel,
            out_shape=jax.ShapeDtypeStruct((B, D), A_x.dtype),
            in_specs=[pl.BlockSpec(memory_space=pltpu.HBM)] * len(args),
            scratch_shapes=[
                pltpu.VMEM((B, D), bf16), pltpu.VMEM((B, D), bf16), pltpu.VMEM(w_mod.shape, bf16),
                pltpu.VMEM(A_wq.shape, bf16), pltpu.VMEM(A_wo.shape, bf16),
                pltpu.VMEM((F, D), bf16), pltpu.VMEM((F, D), bf16), pltpu.VMEM((F, D), bf16),
                pltpu.VMEM((NC, G, R, DH), bf16), pltpu.VMEM((NC, G, R, DH), bf16),
                pltpu.VMEM((NG, G, DH), f32), pltpu.VMEM((NC, G, R), f32), pltpu.VMEM((NC, G, R), bf16),
                pltpu.VMEM((G, DH), f32), pltpu.VMEM((NG, G, DH), f32),
                pltpu.SemaphoreType.DMA((10,)), pltpu.SemaphoreType.DMA((NC,)),
                pltpu.SemaphoreType.DMA((NC,)),
            ],
            compiler_params=pltpu.CompilerParams(
                vmem_limit_bytes=96 * 1024 * 1024, disable_bounds_checks=not checks),
        )(*args)
        return out.reshape(B, Sq, D)

    return f


_impl = make()


@jax.jit
def pallas_adaLN_cond__sliding_block_cached__glu_gated_swiglu__decode_kernel(
    A_x, A_k_cache, A_v_cache, A_wq, A_wo, B_x, B_w1, B_w3, B_w2, c, w_mod,
):
    return _impl(A_x, A_k_cache, A_v_cache, A_wq, A_wo, B_x, B_w1, B_w3, B_w2, c, w_mod)
```

```python
import jax
import jax.numpy as jnp
import jax.experimental.pallas as pl
import jax.experimental.pallas.tpu as pltpu

NT = (((1,), (1,)), ((), ()))
f32 = jnp.float32
bf16 = jnp.bfloat16
G = 8
A = 2
PIECE = 64
STEP = 128
WAYS = 8
WROWS = 32


def _ln(x, eps=1e-5):
    m = jnp.mean(x, axis=-1, keepdims=True)
    d = x - m
    v = jnp.mean(d * d, axis=-1, keepdims=True)
    return d / jnp.sqrt(v + eps)


def _spread(items):
    per = -(-len(items) // WAYS)
    return [items[w * per + j] for j in range(per) for w in range(WAYS) if w * per + j < len(items)]


def _loop(n, body):
    jax.lax.fori_loop(0, n, lambda i, c: (body(i), c)[1], 0)


def _start(copies, pat=(0, 1)):
    for i, cp in enumerate(copies):
        cp.start(priority=pat[i % len(pat)])


def _wait(dst, sem):
    pltpu.make_async_copy(dst, dst, sem).wait()


def _ds(start, size, mult):
    return pl.ds(start if isinstance(start, int) else pl.multiple_of(start, mult), size)


def _rows8(ref):
    v = ref[...].astype(f32)
    row = jax.lax.broadcasted_iota(jnp.int32, (8, v.shape[1]), 0)
    return jnp.where(row == 0, v[0:1], v[1:2])


def make(d=2, lag=8, off=1, nwo=4, wso=64, wsq=16, wsm=64, checks=False, nosem=False, scoped=False,
         plast=(0, 1)):
    def kernel(x_hbm, k_hbm, v_hbm, wq_hbm, wo_hbm, w1_hbm, w3_hbm, w2_hbm, c_hbm, wm_hbm,
               o_ref,
               kbuf, vbuf, xv, cv, wpv, wov, w13v, w2v, lhs, res, qw, ss, ps, acc, os_, gu, hf, ys, sem):
        NS, NA, NM, ND, SK, DH = k_hbm.shape
        B, D = xv.shape
        H = NS * G // B
        W = kbuf.shape[4]
        R = A * STEP
        NI = W // STEP
        NG = NS // A
        F = w2_hbm.shape[0]
        FP = w13v.shape[1]
        NF = FP // D
        FL = F - (NF - 1) * D
        NQ = wq_hbm.shape[1] // D
        hpb = D // DH
        s_a, s_k, s_v, s_g = 0, 1, 3, 5
        HALF = NI // 2
        assert NF <= 3
        cur = [None]

        def mark(name):
            if not scoped:
                return
            if cur[0] is not None:
                cur[0].__exit__(None, None, None)
                cur[0] = None
            if name:
                cur[0] = jax.named_scope(name)
                cur[0].__enter__()

        def copy(src, dst, s, r, nr, sc, dc, nc):
            return pltpu.make_async_copy(src.at[_ds(r, nr, 8), _ds(sc, nc, 128)],
                                         dst.at[_ds(r, nr, 8), _ds(dc, nc, 128)], sem.at[s])

        def start_kv(hbm, buf, s, g, i):
            _start([pltpu.make_async_copy(
                        hbm.at[g * A + a, n, :, j, _ds(SK - W + i * STEP + r, PIECE, PIECE)],
                        buf.at[a, n, :, j, _ds(i * STEP + r, PIECE, PIECE)], sem.at[s + i // HALF])
                    for r in range(0, STEP, PIECE) for a in range(A) for n in range(NA) for j in range(ND)])

        def wait_kv(buf, s, i):
            @pl.when(i % HALF == 0)
            def _():
                _wait(buf.at[:, :, :, :, _ds(i * STEP, W // 2, W // 2)], sem.at[s + i // HALF])

        def head(buf, a, c, w):
            return buf[a, w // (NM * ND), w // ND % NM, w % ND, _ds(c * R, R, R), :]

        def wayrow(w, i, rows, stride):
            per = stride // rows
            return (i // per) * (stride * WAYS) + w * stride + (i % per) * rows

        mark("P0")
        cc = pltpu.make_async_copy(c_hbm, cv, sem.at[s_a])
        cx = pltpu.make_async_copy(x_hbm, xv, sem.at[s_a])
        _start([cc, cx])

        def start_cols(src, s, dc, ncols, stride):
            half = ncols // 2
            _loop(2 * D // (8 * WAYS), lambda t: _start(
                [copy(src, wpv, s, wayrow(w, t // 2, 8, stride), 8, (t % 2) * half, dc + (t % 2) * half, half)
                 for w in range(WAYS)]))

        start_cols(wm_hbm, s_a, 0, 5 * D, wsm)
        start_cols(wq_hbm, s_v + 1, 5 * D, NQ * D, wsq)
        for buf in (w13v.at[0], w13v.at[1], w2v):
            buf[F:FP, :] = jnp.zeros((FP - F, D), bf16)

        def pro_body(i):
            start_kv(k_hbm, kbuf, s_k, 0, i)
            j = i - off

            @pl.when(j == 0)
            def _():
                cc.wait()
                cx.wait()
                _wait(wpv.at[:, pl.ds(0, 5 * D)], sem.at[s_a])
                cf = _rows8(cv)
                sc = (cf * jax.nn.sigmoid(cf)).astype(bf16)
                lhs[...] = sc
                hf[NF] = sc

            @pl.when(j == 5)
            def _():
                _wait(wpv.at[:, pl.ds(5 * D, NQ * D)], sem.at[s_v + 1])
                lhs[...] = (_ln(_rows8(xv)) * (1.0 + res[1]) + res[0]).astype(bf16)

            @pl.when(jnp.logical_and(j >= 0, j < 5 + NQ))
            def _():
                res[j] = jnp.dot(lhs[...], wpv[:, _ds(j * D, D, D)], preferred_element_type=f32)

        _loop(NI, pro_body)

        scale = DH ** -0.5
        row = jax.lax.broadcasted_iota(jnp.int32, (G, DH), 0)
        n_wo = wo_hbm.shape[0] // (WAYS * WROWS)
        way_full = D // (WAYS // 2)
        way_last = FL // (WAYS // 2)
        rpb = way_full // WROWS
        n_13 = (NF - 1) * rpb + way_last // WROWS

        def start_weights(i):
            @pl.when(i < n_wo)
            def _():
                _start([copy(wo_hbm, wov, s_a, wayrow(w, i, WROWS, wso), WROWS, 0, 0, D) for w in range(WAYS)])

            def start_13(j, way, r, nr):
                _start([copy(src, w13v.at[n], 1 + j, j * D + w * way + r, nr, 0, 0, D)
                        for w in range(WAYS // 2) for n, src in enumerate((w1_hbm, w3_hbm))])

            t = i - n_wo

            @pl.when(jnp.logical_and(t >= 0, t < n_13))
            def _():
                j = t // rpb
                start_13(j, jnp.where(j == NF - 1, way_last, way_full), (t % rpb) * WROWS, WROWS)

            @pl.when(t == n_13)
            def _():
                r = (n_13 % rpb) * WROWS
                start_13(NF - 1, way_last, r, way_last - r)

        def group(g):
            for a in range(A):
                sg = g * A + a
                b = sg // (H // G)
                blk = 5 + (sg % (H // G)) * (G // hpb)
                for n in range(G // hpb):
                    q = res[blk + n]
                    q = jnp.where(b == 0, q[0:1], q[1:2])
                    for h in range(hpb):
                        w = n * hpb + h
                        qw[a, w] = jnp.where(row == w, q[:, h * DH:(h + 1) * DH], 0.0).astype(bf16)

            def k_body(i):
                start_kv(v_hbm, vbuf, s_v, g, i)
                wait_kv(kbuf, s_k, i)
                c, a = i // A, i % A
                s = None
                for w in range(G):
                    t = jax.lax.dot_general(qw[a, w], head(kbuf, a, c, w), NT, preferred_element_type=f32)
                    s = t if s is None else s + t
                ss[a, c] = s * scale

            _loop(NI, k_body)

            def softmax(a):
                s = ss[a]
                m = jnp.max(jnp.max(s, axis=0), axis=-1, keepdims=True)
                p = jnp.exp(s - m)
                l = jnp.sum(jnp.sum(p, axis=0), axis=-1, keepdims=True)
                ps[a] = p.astype(bf16)
                acc[a] = jnp.zeros((G, DH), f32)
                os_[g * A + a] = jnp.broadcast_to(l, (G, DH))

            _loop(A, softmax)

            def v_body(i):
                @pl.when(g < NG - 1)
                def _():
                    start_kv(k_hbm, kbuf, s_k, g + 1, i)

                @pl.when(g == NG - 1)
                def _():
                    start_weights(i)

                wait_kv(vbuf, s_v, i)
                c, a = i // A, i % A
                p = ps[a, c]
                t = acc[a]
                for w in range(G):
                    o = jnp.dot(p, head(vbuf, a, c, w), preferred_element_type=f32)
                    t = t + jnp.where(row == w, o, 0.0)
                acc[a] = t

            _loop(NI, v_body)

            for a in range(A):
                os_[g * A + a] = acc[a] / os_[g * A + a]

        mark("MAIN")
        _loop(NG, group)

        mark("T1_wo")
        last = _spread([copy(w2_hbm, w2v, s_v + 1, r, WROWS, 0, 0, D) for r in range(0, F - FL, WROWS)])
        last += _spread([copy(w2_hbm, w2v, s_a, r, WROWS, 0, 0, D) for r in range(F - FL, F, WROWS)])
        last += _spread([copy(wm_hbm, w2v.at[pl.ds(FP, D)], s_g, r, WROWS, 5 * D, 0, D)
                         for r in range(0, D, WROWS)])
        _wait(wov, sem.at[s_a])

        def wo_body(j, a):
            @pl.when(j == nwo)
            def _():
                _start(last, plast)

            per = G // hpb
            cols = [jnp.where(row == 0,
                              os_[j // per, pl.ds((j % per) * hpb + n, 1), :],
                              os_[H // G + j // per, pl.ds((j % per) * hpb + n, 1), :]) for n in range(hpb)]
            o = jnp.concatenate(cols, axis=-1).astype(bf16)
            return a + jnp.dot(o, wov[_ds(j * D, D, D), :], preferred_element_type=f32)

        attn = jax.lax.fori_loop(0, wov.shape[0] // D, wo_body, jnp.zeros((8, D), f32))
        x1 = _rows8(xv) + res[2] * attn
        res[0] = x1
        lhs[...] = (_ln(x1) * (1.0 + res[4]) + res[3]).astype(bf16)
        mark("T2_gu")

        def gu_body(t):
            n, j = t % 2, t // 2

            @pl.when(jnp.logical_and(n == 0, j < NF - 1))
            def _():
                _wait(w13v.at[:, _ds(j * D, D, D)], sem.at[1 + j])

            @pl.when(t == 2 * (NF - 1))
            def _():
                _wait(w13v.at[:, pl.ds(F - FL, FL)], sem.at[NF])

            r = jax.lax.dot_general(lhs[...], w13v[n, _ds(j * D, D, D), :], NT, preferred_element_type=f32)

            @pl.when(n == 0)
            def _():
                gu[...] = r * jax.nn.sigmoid(r)

            @pl.when(n == 1)
            def _():
                hf[j] = (gu[...] * r).astype(bf16)

        _loop(2 * NF, gu_body)
        mark("T3_y")

        def y_body(j):
            @pl.when(j == 0)
            def _():
                _wait(w2v.at[pl.ds(0, F - FL)], sem.at[s_v + 1])

            @pl.when(j == NF - 1)
            def _():
                _wait(w2v.at[pl.ds(F - FL, FL)], sem.at[s_a])

            @pl.when(j == NF)
            def _():
                _wait(w2v.at[pl.ds(FP, D)], sem.at[s_g])

            ys[j] = jnp.dot(hf[j], w2v[_ds(j * D, D, D), :], preferred_element_type=f32)

        _loop(NF + 1, y_body)
        y = ys[0]
        for j in range(1, NF):
            y = y + ys[j]
        o_ref[...] = (res[0] + ys[NF] * y)[0:B].astype(o_ref.dtype)
        mark(None)

    def f(A_x, A_k_cache, A_v_cache, A_wq, A_wo, B_x, B_w1, B_w3, B_w2, c, w_mod):
        B, Sq, D = A_x.shape
        _, H, SK, DH = A_k_cache.shape
        W = min(4096, max(256, SK // 4))
        F = B_w1.shape[1]
        NF = -(-F // D)
        FP = NF * D
        R = A * STEP
        NS = B * H // G
        NP = 5 + H * DH // D
        hshape = (G // (2 * d), 2, d)
        args = [A_x.reshape(B, D), A_k_cache.reshape(NS, *hshape, SK, DH), A_v_cache.reshape(NS, *hshape, SK, DH),
                A_wq, A_wo, B_w1.T, B_w3.T, B_w2, c, w_mod]
        args = [pltpu.with_memory_space_constraint(a, pltpu.HBM) for a in args]
        out = pl.pallas_call(
            kernel,
            out_shape=jax.ShapeDtypeStruct((B, D), A_x.dtype),
            in_specs=[pl.BlockSpec(memory_space=pltpu.HBM)] * len(args),
            scratch_shapes=[
                pltpu.VMEM((A, *hshape, W, DH), bf16), pltpu.VMEM((A, *hshape, W, DH), bf16),
                pltpu.VMEM((B, D), bf16), pltpu.VMEM((B, D), bf16),
                pltpu.VMEM((D, NP * D), bf16), pltpu.VMEM(A_wo.shape, bf16),
                pltpu.VMEM((2, FP, D), bf16), pltpu.VMEM((FP + D, D), bf16),
                pltpu.VMEM((8, D), bf16), pltpu.VMEM((NP, 8, D), f32),
                pltpu.VMEM((A, G, G, DH), bf16),
                pltpu.VMEM((A, W // R, G, R), f32), pltpu.VMEM((A, W // R, G, R), bf16),
                pltpu.VMEM((A, G, DH), f32), pltpu.VMEM((NS, G, DH), f32),
                pltpu.VMEM((8, D), f32), pltpu.VMEM((NF + 1, 8, D), bf16), pltpu.VMEM((NF + 1, 8, D), f32),
                pltpu.SemaphoreType.DMA((NF + 3,)),
            ],
            compiler_params=pltpu.CompilerParams(
                vmem_limit_bytes=96 * 1024 * 1024, disable_bounds_checks=not checks,
                disable_semaphore_checks=nosem),
        )(*args)
        return out.reshape(B, Sq, D)

    return f


_impl = make(nwo=7, plast=(1, 1, 0))


@jax.jit
def pallas_adaLN_cond__sliding_block_cached__glu_gated_swiglu__decode_kernel(
    A_x, A_k_cache, A_v_cache, A_wq, A_wo, B_x, B_w1, B_w3, B_w2, c, w_mod,
):
    return _impl(A_x, A_k_cache, A_v_cache, A_wq, A_wo, B_x, B_w1, B_w3, B_w2, c, w_mod)
```

```python
import jax
import jax.numpy as jnp
import jax.experimental.pallas as pl
import jax.experimental.pallas.tpu as pltpu

NT = (((1,), (1,)), ((), ()))
f32 = jnp.float32
bf16 = jnp.bfloat16

G = 8
A = 2
PAIR = 2
PIECE = 64
STEP = 128
WAYS = 8
WROWS = 32
NMOD = 5

S_W, S_K, S_V, S_G = 0, 1, 3, 5
N_SEM = 6


def _layernorm(x, eps=1e-5):
    m = jnp.mean(x, axis=-1, keepdims=True)
    d = x - m
    v = jnp.mean(d * d, axis=-1, keepdims=True)
    return d / jnp.sqrt(v + eps)


def _silu(x):
    return x * jax.nn.sigmoid(x)


def _spread(items):
    per = -(-len(items) // WAYS)
    return [items[w * per + j] for j in range(per) for w in range(WAYS) if w * per + j < len(items)]


def _way_row(w, i, rows, stride):
    per = stride // rows
    return (i // per) * (stride * WAYS) + w * stride + (i % per) * rows


def _loop(n, body):
    jax.lax.fori_loop(0, n, lambda i, c: (body(i), c)[1], 0)


def _start(copies, priorities=(0, 1)):
    for i, cp in enumerate(copies):
        cp.start(priority=priorities[i % len(priorities)])


def _wait(dst, sem):
    pltpu.make_async_copy(dst, dst, sem).wait()


def _ds(start, size, multiple):
    return pl.ds(start if isinstance(start, int) else pl.multiple_of(start, multiple), size)


def _rows8(ref):
    v = ref[...].astype(f32)
    row = jax.lax.broadcasted_iota(jnp.int32, (8, v.shape[1]), 0)
    return jnp.where(row == 0, v[0:1], v[1:2])


def _kernel(x_hbm, k_hbm, v_hbm, wq_hbm, wo_hbm, w1_hbm, w3_hbm, w2_hbm, c_hbm, wm_hbm,
            o_ref,
            kbuf, vbuf, xv, cv, wpv, wov, w13v, w2v,
            lhs, res, qw, ss, ps, acc, os_, sg_ref, hf, ys, sem):
    NS, NA, NM, ND, SK, DH = k_hbm.shape
    B, D = xv.shape
    H = NS * G // B
    W = kbuf.shape[4]
    R = A * STEP
    NI = W // STEP
    HALF = NI // 2
    NG = NS // A
    F = w2_hbm.shape[0]
    FP = w13v.shape[1]
    NF = FP // D
    FL = F - (NF - 1) * D
    NQ = wq_hbm.shape[1] // D
    HPB = D // DH
    scale = DH ** -0.5
    row = jax.lax.broadcasted_iota(jnp.int32, (G, DH), 0)

    def copy(src, dst, s, r, nr, sc, dc, nc):
        return pltpu.make_async_copy(src.at[_ds(r, nr, 8), _ds(sc, nc, 128)],
                                     dst.at[_ds(r, nr, 8), _ds(dc, nc, 128)], sem.at[s])

    def start_kv(hbm, buf, s, g, i):
        _start([pltpu.make_async_copy(
                    hbm.at[g * A + a, n, :, j, _ds(SK - W + i * STEP + r, PIECE, PIECE)],
                    buf.at[a, n, :, j, _ds(i * STEP + r, PIECE, PIECE)],
                    sem.at[s + i // HALF])
                for r in range(0, STEP, PIECE) for a in range(A) for n in range(NA) for j in range(ND)])

    def wait_kv(buf, s, i):
        @pl.when(i % HALF == 0)
        def _():
            _wait(buf.at[:, :, :, :, _ds(i * STEP, W // 2, W // 2)], sem.at[s + i // HALF])

    def head(buf, a, c, w):
        return buf[a, w // (NM * ND), w // ND % NM, w % ND, _ds(c * R, R, R), :]

    c_copy = pltpu.make_async_copy(c_hbm, cv, sem.at[S_W])
    x_copy = pltpu.make_async_copy(x_hbm, xv, sem.at[S_W])
    _start([c_copy, x_copy])

    def start_cols(src, s, dc, ncols):
        half = ncols // 2
        _loop(2 * D // (8 * WAYS), lambda t: _start(
            [copy(src, wpv, s, _way_row(w, t // 2, 8, 32), 8, (t % 2) * half, dc + (t % 2) * half, half)
             for w in range(WAYS)]))

    start_cols(wm_hbm, S_W, 0, NMOD * D)
    start_cols(wq_hbm, S_V + 1, NMOD * D, NQ * D)
    for buf in (w13v.at[0], w13v.at[1], w2v):
        buf[F:FP, :] = jnp.zeros((FP - F, D), bf16)

    def prologue(i):
        start_kv(k_hbm, kbuf, S_K, 0, i)
        j = i - 1

        @pl.when(j == 0)
        def _():
            c_copy.wait()
            x_copy.wait()
            _wait(wpv.at[:, pl.ds(0, NMOD * D)], sem.at[S_W])
            sc = _silu(_rows8(cv)).astype(bf16)
            lhs[...] = sc
            hf[NF] = sc

        @pl.when(j == NMOD)
        def _():
            _wait(wpv.at[:, pl.ds(NMOD * D, NQ * D)], sem.at[S_V + 1])
            lhs[...] = (_layernorm(_rows8(xv)) * (1.0 + res[1]) + res[0]).astype(bf16)

        @pl.when(jnp.logical_and(j >= 0, j < NMOD + NQ))
        def _():
            res[j] = jnp.dot(lhs[...], wpv[:, _ds(j * D, D, D)], preferred_element_type=f32)

    _loop(NI, prologue)

    n_wo = wo_hbm.shape[0] // (WAYS * WROWS)
    way_full = D // (WAYS // 2)
    way_last = FL // (WAYS // 2)
    per_block = way_full // WROWS
    n_13 = (NF - 1) * per_block + way_last // WROWS
    assert NF <= 3 and n_wo >= HALF and n_wo + n_13 < NI and NMOD + 1 < HALF
    assert way_last % 8 == 0 and 0 < way_last % WROWS and FL == way_last * (WAYS // 2)

    def start_weights(i):
        @pl.when(i < n_wo)
        def _():
            _start([copy(wo_hbm, wov, S_W, _way_row(w, i, WROWS, 256), WROWS, 0, 0, D) for w in range(WAYS)])

        def start_13(j, way, r, nr):
            _start([copy(src, w13v.at[n], S_K + j, j * D + w * way + r, nr, 0, 0, D)
                    for w in range(WAYS // 2) for n, src in enumerate((w1_hbm, w3_hbm))])

        t = i - n_wo

        @pl.when(jnp.logical_and(t >= 0, t < n_13))
        def _():
            j = t // per_block
            start_13(j, jnp.where(j == NF - 1, way_last, way_full), (t % per_block) * WROWS, WROWS)

        @pl.when(t == n_13)
        def _():
            r = (n_13 % per_block) * WROWS
            start_13(NF - 1, way_last, r, way_last - r)

    def group(g):
        for a in range(A):
            sub = g * A + a
            b = sub // (H // G)
            blk = NMOD + (sub % (H // G)) * (G // HPB)
            for n in range(G // HPB):
                q = res[blk + n]
                q = jnp.where(b == 0, q[0:1], q[1:2])
                for h in range(HPB):
                    w = n * HPB + h
                    qw[a, w] = jnp.where(row == w, q[:, h * DH:(h + 1) * DH], 0.0).astype(bf16)

        def scores(i):
            start_kv(v_hbm, vbuf, S_V, g, i)
            wait_kv(kbuf, S_K, i)
            c, a = i // A, i % A
            s = None
            for w in range(G):
                t = jax.lax.dot_general(qw[a, w], head(kbuf, a, c, w), NT, preferred_element_type=f32)
                s = t if s is None else s + t
            ss[a, c] = s * scale

        _loop(NI, scores)

        def softmax(a):
            s = ss[a]
            m = jnp.max(jnp.max(s, axis=0), axis=-1, keepdims=True)
            p = jnp.exp(s - m)
            l = jnp.sum(jnp.sum(p, axis=0), axis=-1, keepdims=True)
            ps[a] = p.astype(bf16)
            acc[a] = jnp.zeros((G, DH), f32)
            os_[g * A + a] = jnp.broadcast_to(l, (G, DH))

        _loop(A, softmax)

        def values(i):
            @pl.when(g < NG - 1)
            def _():
                start_kv(k_hbm, kbuf, S_K, g + 1, i)

            @pl.when(g == NG - 1)
            def _():
                start_weights(i)

            wait_kv(vbuf, S_V, i)
            c, a = i // A, i % A
            p = ps[a, c]
            t = acc[a]
            for w in range(G):
                o = jnp.dot(p, head(vbuf, a, c, w), preferred_element_type=f32)
                t = t + jnp.where(row == w, o, 0.0)
            acc[a] = t

        _loop(NI, values)
        for a in range(A):
            os_[g * A + a] = acc[a] / os_[g * A + a]

    _loop(NG, group)

    last = _spread([copy(w2_hbm, w2v, S_V + 1, r, WROWS, 0, 0, D) for r in range(0, F - FL, WROWS)])
    last += _spread([copy(w2_hbm, w2v, S_W, r, WROWS, 0, 0, D) for r in range(F - FL, F, WROWS)])
    last += _spread([copy(wm_hbm, w2v.at[pl.ds(FP, D)], S_G, r, WROWS, NMOD * D, 0, D)
                     for r in range(0, D, WROWS)])
    _wait(wov, sem.at[S_W])
    NO = wov.shape[0] // D

    def out_proj(j, total):
        @pl.when(j == NO - 2)
        def _():
            _start(last, (1, 1, 0))

        per = G // HPB
        heads = [jnp.where(row == 0,
                           os_[j // per, pl.ds((j % per) * HPB + n, 1), :],
                           os_[H // G + j // per, pl.ds((j % per) * HPB + n, 1), :]) for n in range(HPB)]
        o = jnp.concatenate(heads, axis=-1).astype(bf16)
        return total + jnp.dot(o, wov[_ds(j * D, D, D), :], preferred_element_type=f32)

    attn = jax.lax.fori_loop(0, NO, out_proj, jnp.zeros((8, D), f32))
    x1 = _rows8(xv) + res[2] * attn
    res[0] = x1
    lhs[...] = (_layernorm(x1) * (1.0 + res[4]) + res[3]).astype(bf16)

    def gate_up(t):
        n, j = t % 2, t // 2

        @pl.when(jnp.logical_and(n == 0, j < NF - 1))
        def _():
            _wait(w13v.at[:, _ds(j * D, D, D)], sem.at[S_K + j])

        @pl.when(t == 2 * (NF - 1))
        def _():
            _wait(w13v.at[:, pl.ds(F - FL, FL)], sem.at[S_K + NF - 1])

        r = jax.lax.dot_general(lhs[...], w13v[n, _ds(j * D, D, D), :], NT, preferred_element_type=f32)

        @pl.when(n == 0)
        def _():
            sg_ref[...] = _silu(r)

        @pl.when(n == 1)
        def _():
            hf[j] = (sg_ref[...] * r).astype(bf16)

    _loop(2 * NF, gate_up)

    def down(j):
        @pl.when(j == 0)
        def _():
            _wait(w2v.at[pl.ds(0, F - FL)], sem.at[S_V + 1])

        @pl.when(j == NF - 1)
        def _():
            _wait(w2v.at[pl.ds(F - FL, FL)], sem.at[S_W])

        @pl.when(j == NF)
        def _():
            _wait(w2v.at[pl.ds(FP, D)], sem.at[S_G])

        ys[j] = jnp.dot(hf[j], w2v[_ds(j * D, D, D), :], preferred_element_type=f32)

    _loop(NF + 1, down)
    y = ys[0]
    for j in range(1, NF):
        y = y + ys[j]
    o_ref[...] = (res[0] + ys[NF] * y)[0:B].astype(o_ref.dtype)


@jax.jit
def pallas_adaLN_cond__sliding_block_cached__glu_gated_swiglu__decode_kernel(
    A_x: jax.Array,
    A_k_cache: jax.Array,
    A_v_cache: jax.Array,
    A_wq: jax.Array,
    A_wo: jax.Array,
    B_x: jax.Array,
    B_w1: jax.Array,
    B_w3: jax.Array,
    B_w2: jax.Array,
    c: jax.Array,
    w_mod: jax.Array,
):
    del B_x
    B, Sq, D = A_x.shape
    _, H, SK, DH = A_k_cache.shape
    W = min(4096, max(256, SK // 4))
    F = B_w1.shape[1]
    NF = -(-F // D)
    FP = NF * D
    R = A * STEP
    NS = B * H // G
    NP = NMOD + H * DH // D
    assert B == 2 and Sq == 1 and A_wq.shape[1] == H * DH and F % WROWS == 0 and F < FP
    heads = (G // (2 * PAIR), 2, PAIR)

    args = [A_x.reshape(B, D), A_k_cache.reshape(NS, *heads, SK, DH), A_v_cache.reshape(NS, *heads, SK, DH),
            A_wq, A_wo, B_w1.T, B_w3.T, B_w2, c, w_mod]
    out = pl.pallas_call(
        _kernel,
        out_shape=jax.ShapeDtypeStruct((B, D), A_x.dtype),
        in_specs=[pl.BlockSpec(memory_space=pltpu.HBM)] * len(args),
        scratch_shapes=[
            pltpu.VMEM((A, *heads, W, DH), bf16),
            pltpu.VMEM((A, *heads, W, DH), bf16),
            pltpu.VMEM((B, D), A_x.dtype),
            pltpu.VMEM((B, D), c.dtype),
            pltpu.VMEM((D, NP * D), bf16),
            pltpu.VMEM(A_wo.shape, bf16),
            pltpu.VMEM((2, FP, D), bf16),
            pltpu.VMEM((FP + D, D), bf16),
            pltpu.VMEM((8, D), bf16),
            pltpu.VMEM((NP, 8, D), f32),
            pltpu.VMEM((A, G, G, DH), bf16),
            pltpu.VMEM((A, W // R, G, R), f32),
            pltpu.VMEM((A, W // R, G, R), bf16),
            pltpu.VMEM((A, G, DH), f32),
            pltpu.VMEM((NS, G, DH), f32),
            pltpu.VMEM((8, D), f32),
            pltpu.VMEM((NF + 1, 8, D), bf16),
            pltpu.VMEM((NF + 1, 8, D), f32),
            pltpu.SemaphoreType.DMA((N_SEM,)),
        ],
        compiler_params=pltpu.CompilerParams(
            vmem_limit_bytes=96 * 1024 * 1024, disable_bounds_checks=True),
    )(*args)
    return out.reshape(B, Sq, D)
```
